```python
import os as _os
_os.environ.setdefault("JAX_PLATFORMS", "cpu")
import jax
import jax.numpy as jnp

def _softmax(x, axis=-1):
    return jax.nn.softmax(x, axis=axis)
def _gelu(x):
    return jax.nn.gelu(x, approximate=True)
def _silu(x):
    return jax.nn.silu(x)
def _sigmoid(x):
    return jax.nn.sigmoid(x)
def _layernorm(x, axis=-1, eps=1e-5):
    m = jnp.mean(x, axis=axis, keepdims=True)
    v = jnp.var(x, axis=axis, keepdims=True)
    return (x - m) / jnp.sqrt(v + eps)
def _scatter_add(tgt, idx, src, axis=0):
    return tgt.at[idx].add(src)
def _segment_sum(src, seg, n):
    return jax.ops.segment_sum(src, seg, n)
class _Rng:
    def __init__(self, key):
        self._k = key
    def _next(self):
        self._k, sub = jax.random.split(self._k)
        return sub
    def normal(self, shape):
        return jax.random.normal(self._next(), shape, dtype=jnp.bfloat16)
    def randint(self, lo, hi, shape):
        return jax.random.randint(self._next(), shape, lo, hi, dtype=jnp.int32)
    def uniform(self, shape, lo=0.0, hi=1.0):
        return jax.random.uniform(self._next(), shape, jnp.bfloat16, lo, hi)
    def permutation(self, n):
        return jax.random.permutation(self._next(), n)


kernel_name = 'standalone__dense_activation_silu__prompt'

def setup_inputs():
    _rng = _Rng(jax.random.key(int.from_bytes(__import__("os").urandom(4), "little")))
    _w = (lambda a: (lambda t: t.astype(jnp.bfloat16) if jnp.issubdtype(t.dtype, jnp.floating) else t)(jnp.asarray(a)))
    B, S, D, F = 1, 2048, 448, 1792
    return {
        "x": _w((lambda *s: _rng.normal(s) * 0.05)(B, S, D)),
        "w1": _w((lambda *s: _rng.normal(s) * 0.05)(D, F) * (D ** -0.5)),
        "w2": _w((lambda *s: _rng.normal(s) * 0.05)(F, D) * (F ** -0.5)),
    }

def reference(x, w1, w2):
    h = jnp.einsum("bsd,df->bsf", x, w1)
    h = _silu(h)
    out = jnp.einsum("bsf,fd->bsd", h, w2)
    return out
```

```python
import jax, jax.numpy as jnp
from jax import lax
from jax.experimental import pallas as pl
from jax.experimental.pallas import tpu as pltpu

bf16, f32 = jnp.bfloat16, jnp.float32
S, D, F, DP, T = 2048, 448, 1792, 512, 128
FLAG = {"XLA_TPU_RESCHEDULE_DMA_DONES": True}

def silu(h):
    return h * pltpu.reciprocal(1.0 + jnp.exp2(h * -1.4426950408889634), approx=True)

def build(prog, flags=FLAG):
    loads = [op[1:4] for op in prog if op[0] == 'ld']
    place, gsize = {}, {}
    for op in prog:
        if op[0] == 'ld':
            g = op[4]
            place[op[1:4]] = (g, gsize.get(g, 0))
            gsize[g] = gsize.get(g, 0) + op[3] - op[2]
    groups = sorted(gsize)
    outs = [(op[1], op[2], op[5], op[6]) for op in prog if op[0] == 'm2']
    outs = sorted(set(outs))
    def kern(xT, w1, w2T, oT, *scr):
        hbm = {'x': xT, 'w1': w1, 'w2': w2T}
        gbuf = dict(zip(groups, scr[:len(groups)]))
        w1T, ob, isem, osem = scr[len(groups):]
        def ld(kind, lo, hi):
            g, off = place[(kind, lo, hi)]
            return pltpu.make_async_copy(hbm[kind].at[:, pl.ds(lo, hi - lo)], gbuf[g].at[pl.ds(0, D), pl.ds(off, hi - lo)], isem.at[loads.index((kind, lo, hi))])
        def st(tlo, thi, dlo, dhi):
            idx = (pl.ds(dlo, dhi - dlo), pl.ds(tlo, thi - tlo))
            return pltpu.make_async_copy(ob.at[idx], oT.at[idx], osem.at[outs.index((tlo, thi, dlo, dhi))])
        def cols(kind, lo, hi, rows):
            parts = []
            for (k, a_, b_) in sorted(l for l in loads if l[0] == kind):
                l, h = max(lo, a_), min(hi, b_)
                if l < h:
                    g, off = place[(k, a_, b_)]
                    parts.append(gbuf[g][rows, pl.ds(off + l - a_, h - l)])
            return parts[0] if len(parts) == 1 else jnp.concatenate(parts, axis=1)
        a, acc, cov, started = {}, {}, {}, []
        for op in prog:
            if op[0] == 'ld':
                ld(*op[1:4]).start()
            elif op[0] == 'z':
                for g in groups:
                    if any(k[0] != 'w2' and place[k][0] == g for k in loads):
                        gbuf[g][pl.ds(D, DP - D), :] = jnp.zeros((DP - D, gsize[g]), bf16)
            elif op[0] == 'wt':
                ld(*op[1:4]).wait()
            elif op[0] == 'tr':
                _, lo, hi = op
                w1T[pl.ds(lo, hi - lo), :] = cols('w1', lo, hi, slice(None)).T
            elif op[0] == 'm1':
                _, tlo, thi, flo, fhi = op
                h = jnp.dot(w1T[pl.ds(flo, fhi - flo), :], cols('x', tlo, thi, slice(None)), preferred_element_type=f32)
                v = silu(h).astype(bf16)
                for fi in range(flo, fhi, T):
                    for ti in range(tlo, thi, T):
                        a[(ti, fi)] = v[fi - flo:fi - flo + T, ti - tlo:ti - tlo + T]
            elif op[0] == 'm2':
                _, tlo, thi, flo, fhi, dlo, dhi = op
                rhs = jnp.concatenate([jnp.concatenate([a[(ti, fi)] for ti in range(tlo, thi, T)], axis=1) for fi in range(flo, fhi, T)], axis=0)
                p = jnp.dot(cols('w2', flo, fhi, pl.ds(dlo, dhi - dlo)), rhs, preferred_element_type=f32)
                key = (tlo, thi, dlo, dhi)
                acc[key] = p if key not in acc else acc[key] + p
                cov[key] = cov.get(key, 0) + fhi - flo
                if cov[key] == F:
                    ob[pl.ds(dlo, dhi - dlo), pl.ds(tlo, thi - tlo)] = acc.pop(key).astype(bf16)
                    st(*key).start(); started.append(key)
        assert not acc and sorted(started) == outs
        for key in started:
            st(*key).wait()
    scratch = [pltpu.VMEM((DP, gsize[g]), bf16) for g in groups]
    scratch += [pltpu.VMEM((F, DP), bf16), pltpu.VMEM((D, S), bf16), pltpu.SemaphoreType.DMA((len(loads),)), pltpu.SemaphoreType.DMA((len(outs),))]
    def f(x, w1, w2):
        B, S_, D_ = x.shape
        xT = pltpu.with_memory_space_constraint(x.reshape(B * S_, D_).T, pltpu.HBM)
        w1 = pltpu.with_memory_space_constraint(w1, pltpu.HBM)
        w2T = pltpu.with_memory_space_constraint(w2.T, pltpu.HBM)
        oT = pl.pallas_call(kern,
            in_specs=[pl.BlockSpec(memory_space=pltpu.HBM)] * 3,
            out_specs=pl.BlockSpec(memory_space=pltpu.HBM),
            out_shape=pltpu.HBM((D_, B * S_), x.dtype),
            scratch_shapes=scratch,
            compiler_params=pltpu.CompilerParams(vmem_limit_bytes=100 * 1024 * 1024, flags=flags),
        )(xT, w1, w2T)
        return oT.T.reshape(B, S_, D_)
    return f

def pairs(sizes, start=0):
    e = [start]
    for c in sizes: e.append(e[-1] + c)
    return list(zip(e[:-1], e[1:]))

def steady(t0, tm=256, fs=(896, 896), pending=(), last_split=(0, 448), inject=None):
    prog = []
    q = list(pending)
    cells = [(t, f) for t in range(t0, S, tm) for f in pairs(fs)]
    for n, (t, f) in enumerate(cells):
        prog.append(('m1', t, t + tm, *f))
        if inject and n in inject: prog += inject[n]
        if q: prog.append(q.pop(0))
        if t + tm == S and len(last_split) > 2:
            continue
        q.append(('m2', t, t + tm, *f, 0, D))
    prog += q
    if len(last_split) > 2:
        for dlo, dhi in zip(last_split[:-1], last_split[1:]):
            prog.append(('m2', S - tm, S, 0, F, dlo, dhi))
    return prog

def p1(w1s=(256,) * 7, w2s=(768, 1024), last_split=(0, 336, 448), fs=(896, 896), nx=1):
    w1c, w2c = pairs(w1s), pairs(w2s)
    prog = [('ld', 'w1', *w1c[0], 'w1'), ('ld', 'x', 0, 256, 'x'), ('ld', 'x', 256, 512, 'x')]
    prog += [('ld', 'w1', *c, 'x' if i < nx else 'w1') for i, c in enumerate(w1c[1:])]
    prog += [('ld', 'w2', *w2c[0], 'w2'), ('ld', 'x', 512, 768, 'x')]
    prog += [('ld', 'w2', *c, 'w2') for c in w2c[1:]]
    prog += [('ld', 'x', 768, S, 'x'), ('z',)]
    prog += [('wt', 'w1', *w1c[0]), ('tr', *w1c[0]), ('wt', 'x', 0, 256), ('m1', 0, 256, *w1c[0]), ('wt', 'x', 256, 512), ('m1', 256, 512, *w1c[0])]
    for c in w1c[1:]:
        prog += [('wt', 'w1', *c), ('tr', *c), ('m1', 0, 512, *c)]
    for i, c in enumerate(w2c):
        prog += [('wt', 'w2', *c)]
        if i == 0: prog += [('wt', 'x', 512, 768)]
        prog += [('m2', 0, 256, *c, 0, D)]
    prog += [('m2', 256, 512, 0, fs[0], 0, D)]
    prog += steady(512, pending=[('m2', 256, 512, fs[0], F, 0, D)], last_split=last_split, fs=fs, inject={0: [('wt', 'x', 768, S)]})
    return prog

def p2(last_split=(0, 336, 448), fs=(896, 896), n0=768, m2fs=(896, 896)):
    c = pairs((256,) * 7)
    xs = pairs((256,) * (n0 // 256))
    prog = [('ld', 'w1', *c[0], 'x'), ('ld', 'x', *xs[0], 'x'), ('ld', 'x', *xs[1], 'x'), ('ld', 'w1', *c[1], 'x')]
    prog += [('ld', 'x', *x, 'x') for x in xs[2:]]
    prog += [('ld', 'w1', *k, 'x') for k in c[2:]]
    prog += [('ld', 'w2', 0, F, 'w2'), ('ld', 'x', n0, S, 'x'), ('z',)]
    prog += [('wt', 'w1', *c[0]), ('tr', *c[0]), ('wt', 'x', *xs[0]), ('m1', *xs[0], *c[0]), ('wt', 'x', *xs[1]), ('m1', *xs[1], *c[0])]
    prog += [('wt', 'w1', *c[1]), ('tr', *c[1])]
    for x in xs[2:]:
        prog += [('wt', 'x', *x), ('m1', *x, *c[0])]
    for i in range(1, 7):
        if i + 1 < 7: prog += [('wt', 'w1', *c[i + 1]), ('tr', *c[i + 1])]
        else: prog += [('wt', 'w2', 0, F)]
        prog += [('m1', 0, n0, *c[i])]
    prog += [('wt', 'x', n0, S)]
    pend = [('m2', *x, *f, 0, D) for x in xs for f in pairs(m2fs)]
    prog += pend[:-1]
    prog += steady(n0, pending=pend[-1:], last_split=last_split, fs=fs)
    return prog

@jax.jit
def pallas_standalone__dense_activation_silu__prompt_kernel(x, w1, w2):
    return build(p2())(x, w1, w2)
```

```python
import jax
import jax.numpy as jnp
from jax.experimental import pallas as pl
from jax.experimental.pallas import tpu as pltpu

S, D, F = 2048, 448, 1792
T = 128
DP = 512

HEAD = 512
NEXT = 768
HEAD_SLICES = (
    (0, 128, (384, 384, 512, 512)),
    (128, 256, (512, 512, 768)),
    (256, DP, (512, 512, 768)),
)
TAIL_ROWS = (0, 256, 352, 416, 448)
NUM_LOAD_SEMS = 7
NEG_LOG2E = -1.4426950408889634


def _silu(h):
    d = 1.0 + jnp.exp2(h * NEG_LOG2E)
    r = pltpu.reciprocal(d, approx=True)
    return h * jnp.where(r > 0.0, r * (2.0 - d * r), r)


def _ffn_kernel(
    xt_hbm,
    w1_hbm,
    w2t_hbm,
    ot_hbm,
    xw_ref,
    w2_ref,
    w1t_ref,
    w2t_ref,
    ot_ref,
    load_sems,
    store_sem,
):
    def piece(hbm, vmem, col0, rows, cols):
        r = pl.ds(rows[0], rows[1] - rows[0])
        n = cols[1] - cols[0]
        return hbm.at[r, pl.ds(cols[0], n)], vmem.at[r, pl.ds(col0 + cols[0], n)]

    def x_piece(rows, cols):
        return piece(xt_hbm, xw_ref, 0, rows, cols)

    def w1_piece(rows, cols):
        return piece(w1_hbm, xw_ref, S, rows, cols)

    head_steps = []
    queue = []
    for k0, k1, widths in HEAD_SLICES:
        rows, f0 = (k0, min(k1, D)), 0
        for width in widths:
            w = w1_piece(rows, (f0, f0 + width))
            if f0 > 0:
                queue.append([w])
            elif k0 > 0:
                queue.append([x_piece(rows, (0, HEAD)), w])
            else:
                queue += [[w], [x_piece(rows, (0, HEAD))]]
            head_steps.append((k0, k1, f0, f0 + width))
            f0 += width
    queue.append([x_piece((0, D), (HEAD, NEXT))])
    queue.append([piece(w2t_hbm, w2_ref, 0, (0, D), (0, F))])
    queue.append([x_piece((0, D), (NEXT, S))])

    def copies(i):
        sem = load_sems.at[i % NUM_LOAD_SEMS]
        return [pltpu.make_async_copy(src, dst, sem) for src, dst in queue[i]]

    waited = []

    def wait_next():
        i = len(waited)
        waited.append(i)
        for copy in copies(i):
            copy.wait()
        if i + NUM_LOAD_SEMS < len(queue):
            for copy in copies(i + NUM_LOAD_SEMS):
                copy.start()

    def fence(ref, value):
        ref[pl.ds(0, 16), pl.ds(ref.shape[1] - T, T)] = value[:16, :T].astype(ref.dtype)

    partial_h = {}
    act = {}
    stores = []

    def transpose_w1(k0, k1, f0, f1):
        value = xw_ref[pl.ds(k0, k1 - k0), pl.ds(S + f0, f1 - f0)].T
        w1t_ref[pl.ds(f0 // 2, (f1 - f0) // 2), pl.ds(k0, k1 - k0)] = pltpu.bitcast(
            value, jnp.uint32
        )
        return value

    def up(t0, t1, f0, f1, k0=0, k1=DP):
        lhs = pltpu.bitcast(
            w1t_ref[pl.ds(f0 // 2, (f1 - f0) // 2), pl.ds(k0, k1 - k0)], jnp.bfloat16
        )
        rhs = xw_ref[pl.ds(k0, k1 - k0), pl.ds(t0, t1 - t0)]
        h = jnp.dot(lhs, rhs, preferred_element_type=jnp.float32)
        for f in range(f0, f1, T):
            for t in range(t0, t1, T):
                tile = h[f - f0 : f - f0 + T, t - t0 : t - t0 + T]
                if k0 > 0:
                    tile = partial_h.pop((t, f)) + tile
                if k1 < DP:
                    partial_h[t, f] = tile
                else:
                    act[t, f] = _silu(tile).astype(jnp.bfloat16)

    def down(t0, t1, d0=0, d1=D):
        rhs = jnp.concatenate(
            [
                jnp.concatenate([act[t, f] for t in range(t0, t1, T)], axis=1)
                for f in range(0, F, T)
            ],
            axis=0,
        )
        lhs = pltpu.bitcast(w2t_ref[pl.ds(d0 // 2, (d1 - d0) // 2), :], jnp.bfloat16)
        out = jnp.dot(lhs, rhs, preferred_element_type=jnp.float32)
        idx = (pl.ds(d0, d1 - d0), pl.ds(t0, t1 - t0))
        ot_ref[idx] = out.astype(ot_ref.dtype)
        store = pltpu.make_async_copy(ot_ref.at[idx], ot_hbm.at[idx], store_sem)
        store.start()
        stores.append(store)

    for i in range(NUM_LOAD_SEMS):
        for copy in copies(i):
            copy.start()
    xw_ref[pl.ds(D, DP - D), pl.ds(0, S + F)] = jnp.zeros((DP - D, S + F), xw_ref.dtype)

    wait_next()
    fence(xw_ref, transpose_w1(*head_steps[0])[-16:])
    wait_next()
    for n, (k0, k1, f0, f1) in enumerate(head_steps):
        up(0, HEAD, f0, f1, k0, k1)
        fence(xw_ref, partial_h[0, f0] if k1 < DP else act[0, f0])
        wait_next()
        if n + 1 < len(head_steps):
            transpose_w1(*head_steps[n + 1])

    up(HEAD, NEXT, 0, F // 2)
    fence(w2_ref, act[HEAD, 5 * T])
    wait_next()
    w2t_ref[...] = pltpu.bitcast(w2_ref[:, pl.ds(0, F)], jnp.uint32)
    down(0, T)
    down(T, 2 * T)
    up(HEAD, NEXT, F // 2, F)
    wait_next()
    down(2 * T, 3 * T)
    down(3 * T, 4 * T)

    for t in range(NEXT, S, T):
        up(t, t + T, 0, F)
        down(t - 2 * T, t - T)
    for d0, d1 in zip(TAIL_ROWS[:-1], TAIL_ROWS[1:]):
        down(S - 2 * T, S, d0, d1)

    assert len(waited) == len(queue) and not partial_h
    for store in stores:
        store.wait()


@jax.jit
def pallas_standalone__dense_activation_silu__prompt_kernel(
    x: jax.Array,
    w1: jax.Array,
    w2: jax.Array,
):
    assert x.shape == (1, S, D) and w1.shape == (D, F) and w2.shape == (F, D)
    assert x.dtype == w1.dtype == w2.dtype == jnp.bfloat16
    hbm = pl.BlockSpec(memory_space=pltpu.HBM)
    out_t = pl.pallas_call(
        _ffn_kernel,
        in_specs=[hbm, hbm, hbm],
        out_specs=hbm,
        out_shape=jax.ShapeDtypeStruct((D, S), x.dtype),
        scratch_shapes=[
            pltpu.VMEM((DP, S + F + T), jnp.bfloat16),
            pltpu.VMEM((D, F + T), jnp.bfloat16),
            pltpu.VMEM((F // 2, DP), jnp.uint32),
            pltpu.VMEM((D // 2, F), jnp.uint32),
            pltpu.VMEM((D, S), x.dtype),
            pltpu.SemaphoreType.DMA((NUM_LOAD_SEMS,)),
            pltpu.SemaphoreType.DMA(()),
        ],
        compiler_params=pltpu.CompilerParams(
            vmem_limit_bytes=64 * 1024 * 1024,
            flags={"XLA_TPU_RESCHEDULE_DMA_DONES": True},
        ),
    )(x.reshape(S, D).T, w1, w2.T)
    return out_t.T.reshape(1, S, D)
```
